```python
import os as _os
_os.environ.setdefault("JAX_PLATFORMS", "cpu")
import jax
import jax.numpy as jnp

def _softmax(x, axis=-1):
    return jax.nn.softmax(x, axis=axis)
def _gelu(x):
    return jax.nn.gelu(x, approximate=True)
def _silu(x):
    return jax.nn.silu(x)
def _sigmoid(x):
    return jax.nn.sigmoid(x)
def _layernorm(x, axis=-1, eps=1e-5):
    m = jnp.mean(x, axis=axis, keepdims=True)
    v = jnp.var(x, axis=axis, keepdims=True)
    return (x - m) / jnp.sqrt(v + eps)
def _scatter_add(tgt, idx, src, axis=0):
    return tgt.at[idx].add(src)
def _segment_sum(src, seg, n):
    return jax.ops.segment_sum(src, seg, n)
class _Rng:
    def __init__(self, key):
        self._k = key
    def _next(self):
        self._k, sub = jax.random.split(self._k)
        return sub
    def normal(self, shape):
        return jax.random.normal(self._next(), shape, dtype=jnp.bfloat16)
    def randint(self, lo, hi, shape):
        return jax.random.randint(self._next(), shape, lo, hi, dtype=jnp.int32)
    def uniform(self, shape, lo=0.0, hi=1.0):
        return jax.random.uniform(self._next(), shape, jnp.bfloat16, lo, hi)
    def permutation(self, n):
        return jax.random.permutation(self._next(), n)


kernel_name = 'sequential_preLN__mha_block__dense_activation_squared_relu__prompt'

def setup_inputs():
    _rng = _Rng(jax.random.key(int.from_bytes(__import__("os").urandom(4), "little")))
    _w = (lambda a: (lambda t: t.astype(jnp.bfloat16) if jnp.issubdtype(t.dtype, jnp.floating) else t)(jnp.asarray(a)))
    def _A_setup():
        B, S, D, H = 1, 2048, 448, 16
        return {
            "x": _w((lambda *s: _rng.normal(s) * 0.05)(B, S, D)),
            "wqkv": _w((lambda *s: _rng.normal(s) * 0.05)(D, 3 * D)),
            "wo": _w((lambda *s: _rng.normal(s) * 0.05)(D, D)),
        }
    _A_in = _A_setup()

    def _B_setup():
        B, S, D, F = 1, 2048, 448, 1792
        return {
            "x": _w((lambda *s: _rng.normal(s) * 0.05)(B, S, D)),
            "w1": _w((lambda *s: _rng.normal(s) * 0.05)(D, F)),
            "b1": _w((lambda *s: _rng.normal(s) * 0.05)(F)),
            "w2": _w((lambda *s: _rng.normal(s) * 0.05)(F, D)),
            "b2": _w((lambda *s: _rng.normal(s) * 0.05)(D)),
        }
    _B_in = _B_setup()

    return {
        "A_x": _A_in["x"],
        "A_wqkv": _A_in["wqkv"],
        "A_wo": _A_in["wo"],
        "B_x": _B_in["x"],
        "B_w1": _B_in["w1"],
        "B_b1": _B_in["b1"],
        "B_w2": _B_in["w2"],
        "B_b2": _B_in["b2"],
    }

def reference(A_x, A_wqkv, A_wo, B_x, B_w1, B_b1, B_w2, B_b2):
    def _A_ref(x, wqkv, wo):
        B, S, D = x.shape
        H = 16
        Dh = D // H
        qkv = (lambda x, *d: x.transpose(*d))((x @ wqkv).reshape(B, S, 3, H, Dh), 2, 0, 3, 1, 4)
        q, k, v = qkv[0], qkv[1], qkv[2]
        scores = jnp.einsum("bhqd,bhkd->bhqk", q, k) * (Dh ** -0.5)
        p = _softmax(scores, axis=-1)
        o = jnp.einsum("bhqk,bhkd->bhqd", p, v)
        return (lambda x, *d: x.transpose(*d))(o, 0, 2, 1, 3).reshape(B, S, D) @ wo

    def _B_ref(x, w1, b1, w2, b2):
        h = jnp.einsum("bsd,df->bsf", x, w1) + b1
        zero = jnp.zeros_like(h)
        r = jnp.where(h > zero, h, zero)
        h = r * r
        out = jnp.einsum("bsf,fd->bsd", h, w2) + b2
        return out

    x = A_x
    h = x + _A_ref(_layernorm(x, axis=-1), A_wqkv, A_wo)
    h2 = h + _B_ref(_layernorm(h, axis=-1), B_w1, B_b1, B_w2, B_b2)
    return h2
```

```python
import jax
import jax.numpy as jnp
from jax import lax
import jax.experimental.pallas as pl
import jax.experimental.pallas.tpu as pltpu

S = 2048
D = 448
H = 16
DH = 28
DP = 32
G = 112
F = 1792
EPS = 1e-5
LOG2E = 1.4426950408889634
QSCALE = (DH ** -0.5) * LOG2E
f32 = jnp.float32
bf16 = jnp.bfloat16
QW = 48
QOFF = (0, 16, 48, 64)
WPIECES = ((0, 256), (256, 512), (512, 896), (896, 1344))


def _dot(a, b):
    return jnp.dot(a, b, preferred_element_type=f32)


def _ln_t(x):
    m = jnp.mean(x, axis=0, keepdims=True)
    xc = x - m
    v = jnp.mean(xc * xc, axis=0, keepdims=True)
    return xc * lax.rsqrt(v + EPS)


def make_kernel(tq, ck, ne, hp):
    NQ = S // tq
    NC = S // ck
    NI = NQ * H
    te = tq // ne
    NW = len(WPIECES)

    def kernel(x_hbm, wqkv_hbm, wo_hbm, w1_hbm, w2t_hbm, b1_ref, b2_ref,
               o_hbm,
               x_v, wqkv_v, wo_v, w1_v, w2t_v, wall_t, wot, w1t, b2c,
               k_scr, vt_scr, qm_scr, s2_scr, m_scr, ot_scr, otn_scr, o_v, sems, osems):
        i = pl.program_id(0)
        sa_scr = s2_scr.at[0]
        sb_scr = s2_scr.at[1]

        def qk_chunk(a, j, c, s_scr, m):
            g = (a % H) // 4
            parts = []
            if QOFF[j]:
                parts.append(jnp.zeros((QOFF[j], tq), bf16))
            parts.append(qm_scr[a])
            parts.append(jnp.zeros((128 - QW - QOFF[j], tq), bf16))
            qm = jnp.concatenate(parts, axis=0)
            s = _dot(k_scr[g, c * ck:(c + 1) * ck, :], qm)
            s_scr[c * ck:(c + 1) * ck, :] = s
            sm = jnp.max(s.reshape(ck // 8, 8, tq), axis=0)
            return sm if m is None else jnp.maximum(m, sm)

        def pv_chunk(h, c, s_scr, m, acc):
            p = jnp.exp2(s_scr[c * ck:(c + 1) * ck, :] - m).astype(bf16)
            o = _dot(vt_scr[h, :, c * ck:(c + 1) * ck], p)
            return o if acc is None else acc + o

        def fin(m8):
            return jnp.max(m8, axis=0, keepdims=True)

        def normalize(h):
            o = ot_scr[h]
            otn_scr[h] = (o * (1.0 / o[DH:DH + 1, :])).astype(bf16)

        def half(h_b, sb, mb, a, j, sa):
            m = None
            acc = None
            for c in range(NC):
                if a is not None:
                    m = qk_chunk(a, j, c, sa, m)
                if h_b is not None:
                    acc = pv_chunk(h_b, c, sb, mb, acc)
            if h_b is not None:
                ot_scr[h_b] = acc
            return None if m is None else fin(m)

        def out_copy(step, e):
            c0 = step * tq + e * te
            if not isinstance(c0, int):
                c0 = pl.multiple_of(c0, 128)
            return pltpu.make_async_copy(o_v.at[:, pl.ds(c0, te)], o_hbm.at[:, pl.ds(c0, te)],
                                         osems.at[step * ne + e])

        @pl.when(i == 0)
        def _prologue():
            cp_x = [pltpu.make_async_copy(x_hbm.at[:, c * tq:(c + 1) * tq], x_v.at[:, c * tq:(c + 1) * tq],
                                          sems.at[c]) for c in range(NQ)]
            cp_w = [pltpu.make_async_copy(wqkv_hbm.at[:, lo:hi], wqkv_v.at[:, lo:hi], sems.at[NQ + p])
                    for p, (lo, hi) in enumerate(WPIECES)]
            cp_wo = pltpu.make_async_copy(wo_hbm, wo_v, sems.at[NQ + NW])
            cp_w1 = pltpu.make_async_copy(w1_hbm, w1_v, sems.at[NQ + NW + 1])
            cp_w2 = pltpu.make_async_copy(w2t_hbm, w2t_v, sems.at[NQ + NW + 2])
            cp_w[0].start()
            cp_x[0].start()
            for p in range(1, NW):
                cp_w[p].start()
            for c in range(1, NQ):
                cp_x[c].start()
            cp_wo.start()
            cp_w1.start()
            cp_w2.start()

            def prep_w(p):
                lo, hi = WPIECES[p]
                wt = wqkv_v[:, lo:hi].T
                if lo < 2 * D:
                    wall_t[lo:hi, :] = wt
                else:
                    wvt = wt.astype(f32)
                    zpad = jnp.zeros((DP - DH, D), f32)
                    for h in range(H):
                        blk = jnp.concatenate([wvt[DH * h:DH * (h + 1), :], zpad], axis=0)
                        wall_t[2 * D + DP * h:2 * D + DP * (h + 1), :] = blk.astype(bf16)

            def rows_of(p):
                lo, hi = WPIECES[p]
                return (lo, hi) if lo < 2 * D else (lo, 2 * D + H * DP)

            roww = lax.broadcasted_iota(jnp.int32, (QW, tq), 0)
            rowv = lax.broadcasted_iota(jnp.int32, (H * DP, tq), 0)

            def post(c, r):
                for g in range(4):
                    for j in range(4):
                        qw = r[G * g + QOFF[j]:G * g + QOFF[j] + QW, :] * QSCALE
                        lo = DH * j - QOFF[j]
                        msk = (roww >= lo) & (roww < lo + DH)
                        qm_scr[c * H + 4 * g + j] = jnp.where(msk, qw, 0.0).astype(bf16)
                    kg = r[D + G * g:D + G * g + 128, :].astype(bf16)
                    k_scr[g, c * tq:(c + 1) * tq, :] = kg.T
                vt = r[2 * D:, :]
                vt = jnp.where(rowv % DP == DH, 1.0, vt).astype(bf16)
                for h in range(H):
                    vt_scr[h, :, c * tq:(c + 1) * tq] = vt[DP * h:DP * (h + 1), :]

            def ln_x(c):
                return _ln_t(x_v[:, c * tq:(c + 1) * tq].astype(f32)).astype(bf16)

            cp_w[0].wait()
            prep_w(0)
            cp_x[0].wait()
            xn = ln_x(0)
            rs = []
            for p in range(NW):
                if p + 1 < NW:
                    cp_w[p + 1].wait()
                else:
                    for c in range(1, NQ):
                        cp_x[c].wait()
                lo, hi = rows_of(p)
                rs.append(_dot(wall_t[lo:hi, :], xn))
                if p + 1 < NW:
                    prep_w(p + 1)
            post(0, jnp.concatenate(rs, axis=0))
            for c in range(1, NQ):
                post(c, _dot(wall_t[...], ln_x(c)))

            cp_wo.wait()
            cp_w1.wait()
            cp_w2.wait()
            m_scr[...] = half(None, None, None, 0, 0, sa_scr)
            wo32 = wo_v[...].astype(f32)
            zpad = jnp.zeros((DP - DH, D), f32)
            blks = []
            for h in range(H):
                blks.append(wo32[DH * h:DH * (h + 1), :])
                blks.append(zpad)
            wot[...] = jnp.concatenate(blks, axis=0).astype(bf16).T
            r64 = lax.broadcasted_iota(jnp.int32, (64, F), 0)
            b1row = b1_ref[...].reshape(1, F).astype(f32)
            extra = jnp.where(r64 == 0, b1row, 0.0).astype(bf16)
            w1t[...] = jnp.concatenate([w1_v[...], extra], axis=0).T
            b2row = b2_ref[...].reshape(1, D).astype(f32)
            b2c[...] = jnp.broadcast_to(b2row, (128, D)).T

        def hbody(t, m):
            for u in range(hp // 2):
                h = hp * t + 2 * u
                n = i * H + h
                m = half(h, sa_scr, m, n + 1, (2 * u + 1) % 4, sb_scr)
                normalize(h)
                m = half(h + 1, sb_scr, m, (n + 2) % NI, (2 * u + 2) % 4, sa_scr)
                normalize(h + 1)
            return m
        m_scr[...] = lax.fori_loop(0, H // hp, hbody, m_scr[...])

        q0 = pl.multiple_of(i * tq, tq)
        r64 = lax.broadcasted_iota(jnp.int32, (64, te), 0)
        ones_rows = jnp.where(r64 == 0, 1.0, 0.0).astype(bf16)
        hs = []
        for e in range(ne):
            otn = otn_scr[:, :, e * te:(e + 1) * te].reshape(H * DP, te)
            attn = _dot(wot[...], otn)
            hs.append(x_v[:, pl.ds(q0 + e * te, te)].astype(f32) + attn)
        rs = []
        for e in range(ne):
            hn = jnp.concatenate([_ln_t(hs[e]).astype(bf16), ones_rows], axis=0)
            h1 = jnp.maximum(_dot(w1t[...], hn), 0.0)
            rs.append((h1 * h1).astype(bf16))
        b2t = jnp.concatenate([b2c[...]] * (te // 128), axis=1)
        for e in range(ne):
            out = _dot(w2t_v[...], rs[e])
            o_v[:, pl.ds(q0 + e * te, te)] = (hs[e] + b2t + out).astype(bf16)
            out_copy(i, e).start()

        @pl.when(i == NQ - 1)
        def _():
            for s_ in range(NQ):
                for e in range(ne):
                    out_copy(s_, e).wait()
    return kernel


@jax.jit
def pallas_sequential_preLN__mha_block__dense_activation_squared_relu__prompt_kernel(A_x, A_wqkv, A_wo, B_x, B_w1, B_b1, B_w2, B_b2):
    tq = 512
    ck = 128
    ne = 4
    hp = 8
    xt = A_x.reshape(S, D).T
    w2t = B_w2.T
    NQ = S // tq
    anyspec = pl.BlockSpec(memory_space=pl.ANY)
    out = pl.pallas_call(
        make_kernel(tq, ck, ne, hp),
        grid=(NQ,),
        in_specs=[anyspec, anyspec, anyspec, anyspec, anyspec,
                  pl.BlockSpec((F,), lambda i: (0,)), pl.BlockSpec((D,), lambda i: (0,))],
        out_specs=anyspec,
        out_shape=jax.ShapeDtypeStruct((D, S), bf16),
        scratch_shapes=[
            pltpu.VMEM((D, S), bf16),
            pltpu.VMEM((D, 3 * D), bf16),
            pltpu.VMEM((D, D), bf16),
            pltpu.VMEM((D, F), bf16),
            pltpu.VMEM((D, F), bf16),
            pltpu.VMEM((2 * D + H * DP, D), bf16),
            pltpu.VMEM((D, H * DP), bf16),
            pltpu.VMEM((F, 512), bf16),
            pltpu.VMEM((D, 128), f32),
            pltpu.VMEM((4, S, 128), bf16),
            pltpu.VMEM((H, DP, S), bf16),
            pltpu.VMEM((NQ * H, QW, tq), bf16),
            pltpu.VMEM((2, S, tq), f32),
            pltpu.VMEM((1, tq), f32),
            pltpu.VMEM((H, DP, tq), f32),
            pltpu.VMEM((H, DP, tq), bf16),
            pltpu.VMEM((D, S), bf16),
            pltpu.SemaphoreType.DMA((NQ + len(WPIECES) + 3,)),
            pltpu.SemaphoreType.DMA((NQ * ne,)),
        ],
        compiler_params=pltpu.CompilerParams(
            dimension_semantics=("arbitrary",), vmem_limit_bytes=100 * 1024 * 1024),
    )(xt, A_wqkv, A_wo, B_w1, w2t, B_b1, B_b2)
    return out.T.reshape(1, S, D)
```

```python
import jax
import jax.numpy as jnp
from jax import lax
import jax.experimental.pallas as pl
import jax.experimental.pallas.tpu as pltpu

S = 2048
D = 448
H = 16
DH = 28
DP = 32
G = 4 * DH
F = 1792
EPS = 1e-5
LOG2E = 1.4426950408889634
QSCALE = (DH ** -0.5) * LOG2E
f32 = jnp.float32
bf16 = jnp.bfloat16

TQ = 512
CK = 128
NE = 4
HP = 8
LAG = 2
NQ = S // TQ
NC = S // CK
NI = NQ * H
TE = TQ // NE
QW = 48
QOFF = (0, 16, 48, 64)
WPIECES = ((0, 256), (256, 512), (512, 3 * D))


def _dot(a, b):
    return jnp.dot(a, b, preferred_element_type=f32)


def _colmean_fast(x):
    q = x.shape[0] // 4
    s = (x[0:q] + x[q:2 * q]) + (x[2 * q:3 * q] + x[3 * q:])
    return jnp.sum(s, axis=0, keepdims=True) * (1.0 / x.shape[0])


def _colmean(x):
    return jnp.mean(x, axis=0, keepdims=True)


def _ln_t(x, fast=False):
    mean = _colmean_fast if fast else _colmean
    xc = x - mean(x)
    v = mean(xc * xc)
    return xc * lax.rsqrt(v + EPS)


def _kernel(x_hbm, wqkv_hbm, wo_hbm, w1_hbm, w2t_hbm, b1_hbm, b2_hbm,
            o_hbm,
            x_v, wqkv_v, wo_v, w1_v, w2t_v, wall_t, wot, w1t, b2c,
            k_scr, vt_scr, qm_scr, s2_scr, otn_scr, o_v, xn_scr, m_scr, acc_scr,
            b1_v, b2_v, sems):
    i = pl.program_id(0)
    bufs = (s2_scr.at[0], s2_scr.at[1])
    osem = sems.at[7]

    def qk_chunk(a, g, j, c, s_scr, m):
        parts = []
        if QOFF[j]:
            parts.append(jnp.zeros((QOFF[j], TQ), bf16))
        parts.append(qm_scr[a])
        parts.append(jnp.zeros((128 - QW - QOFF[j], TQ), bf16))
        qm = jnp.concatenate(parts, axis=0)
        s = _dot(k_scr[g, c * CK:(c + 1) * CK, :], qm)
        s_scr[c * CK:(c + 1) * CK, :] = s
        sm = jnp.max(s.reshape(CK // 8, 8, TQ), axis=0)
        return sm if m is None else jnp.maximum(m, sm)

    def pv_chunk(h, c, s_scr, m, acc):
        p = jnp.exp2(s_scr[c * CK:(c + 1) * CK, :] - m).astype(bf16)
        o = _dot(vt_scr[h, :, c * CK:(c + 1) * CK], p)
        return o if acc is None else acc + o

    def fin(m8):
        return jnp.max(m8, axis=0, keepdims=True)

    def finish(slot, o):
        otn_scr[slot] = (o * (1.0 / o[DH:DH + 1, :])).astype(bf16)

    @pl.when(i == 0)
    def _prologue():
        def xcopy(lo, hi, sem):
            return pltpu.make_async_copy(x_hbm.at[:, lo:hi], x_v.at[:, lo:hi], sem)

        def wcopy(p, sem):
            lo, hi = WPIECES[p]
            return pltpu.make_async_copy(wqkv_hbm.at[:, lo:hi], wqkv_v.at[:, lo:hi], sem)

        th = TQ // 2
        stage = [
            [wcopy(0, sems.at[0])],
            [xcopy(0, th, sems.at[1])],
            [wcopy(1, sems.at[2]), xcopy(th, TQ, sems.at[2])],
            [wcopy(2, sems.at[3])],
            [xcopy(TQ, 2 * TQ, sems.at[4])],
            [xcopy(2 * TQ, S, sems.at[5])] + [
                pltpu.make_async_copy(src, dst, sems.at[5])
                for src, dst in ((wo_hbm, wo_v), (w1_hbm, w1_v), (b1_hbm, b1_v), (b2_hbm, b2_v))],
            [pltpu.make_async_copy(w2t_hbm, w2t_v, sems.at[6])],
        ]
        for st in stage:
            for cp in st:
                cp.start()

        def wait(k):
            for cp in stage[k]:
                cp.wait()

        def prep_w(p):
            lo, hi = WPIECES[p]
            wall_t[lo:hi, :] = wqkv_v[:, lo:hi].T

        r4 = lax.broadcasted_iota(jnp.int32, (DP - DH, TQ), 0)
        vpad = jnp.where(r4 == 0, 1.0, 0.0)
        kpad = jnp.zeros((128 - G, TQ), bf16)

        def proj(c, lo, hi, xn=None, t0=0, t1=TQ):
            if xn is None:
                xn = xn_scr[:, c * TQ + t0:c * TQ + t1]
            r = _dot(wall_t[lo:hi, :], xn)
            roww = lax.broadcasted_iota(jnp.int32, (QW, t1 - t0), 0)
            for g in range(4):
                if lo <= G * g < hi:
                    for j in range(4):
                        o = G * g + QOFF[j] - lo
                        qw = r[o:o + QW, :] * QSCALE
                        b = DH * j - QOFF[j]
                        msk = (roww >= b) & (roww < b + DH)
                        qm_scr[c * H + 4 * g + j, :, t0:t1] = jnp.where(msk, qw, 0.0).astype(bf16)
            for g in range(4):
                if lo <= D + G * g < hi:
                    o = D + G * g - lo
                    kg = jnp.concatenate([r[o:o + G, :].astype(bf16), kpad], axis=0)
                    k_scr[g, c * TQ:(c + 1) * TQ, :] = kg.T
            for h in range(H):
                if lo <= 2 * D + DH * h < hi:
                    o = 2 * D + DH * h - lo
                    vt = jnp.concatenate([r[o:o + DH, :], vpad], axis=0)
                    vt_scr[h, :, c * TQ:(c + 1) * TQ] = vt.astype(bf16)

        def ln_tile(c0):
            return _ln_t(x_v[:, c0:c0 + 128].astype(f32), c0 == 0).astype(bf16)

        def ln_store(lo, hi):
            for c0 in range(lo, hi, 128):
                xn_scr[:, c0:c0 + 128] = ln_tile(c0)

        bufs[1][...] = jnp.zeros((S, TQ), f32)
        m_scr[...] = jnp.zeros((8, TQ), f32)
        acc_scr[...] = jnp.ones((DP, TQ), f32)

        wait(0)
        prep_w(0)
        wait(1)
        ln_store(0, th)
        proj(0, 0, G, None, 0, th)
        wait(2)
        proj(0, G, 2 * G, None, 0, th)
        prep_w(1)
        proj(0, 2 * G, D, None, 0, th)
        ln_store(th, TQ)
        proj(0, 0, 3 * G, None, th, TQ)
        wait(3)
        proj(0, 3 * G, D, None, th, TQ)
        prep_w(2)
        proj(0, 2 * D, 3 * D)
        wait(4)
        proj(0, D, 2 * D)
        ln_store(TQ, 2 * TQ)
        proj(1, D, 2 * D)
        proj(1, 0, D)
        wait(5)
        proj(1, 2 * D, 3 * D)
        for c in range(2, NQ):
            xn = jnp.concatenate([ln_tile(c0) for c0 in range(c * TQ, (c + 1) * TQ, 128)], axis=1)
            proj(c, 0, 3 * D, xn)

        wo32 = wo_v[...].astype(f32)
        zpad = jnp.zeros((DP - DH, D), f32)
        blks = []
        for h in range(H):
            blks.append(wo32[DH * h:DH * (h + 1), :])
            blks.append(zpad)
        wot[...] = jnp.concatenate(blks, axis=0).astype(bf16).T
        r64 = lax.broadcasted_iota(jnp.int32, (64, F), 0)
        b1row = b1_v[...].reshape(1, F).astype(f32)
        extra = jnp.where(r64 == 0, b1row, 0.0).astype(bf16)
        w1t[...] = jnp.concatenate([w1_v[...], extra], axis=0).T
        b2row = b2_v[...].reshape(1, D).astype(f32)
        b2c[...] = jnp.broadcast_to(b2row, (128, D)).T
        wait(6)

    @pl.when(i < NQ)
    def _attention():
        def hbody(t, carry):
            n0 = i * H + HP * t
            ms = [fin(m_scr[...])]
            finish((n0 - 2) & (2 * H - 1), acc_scr[...])
            accs = {}
            m8 = None

            def do_pv(gb):
                u, c = divmod(gb, NC)
                slot = (n0 + u - 1) & (2 * H - 1)
                accs[u] = pv_chunk(slot & (H - 1), c, bufs[(u + 1) % 2], ms[u], accs.get(u))
                if c == NC - 1:
                    if u == HP - 1:
                        acc_scr[...] = accs[u]
                    else:
                        finish(slot, accs[u])

            for ga in range(HP * NC):
                u, c = divmod(ga, NC)
                m8 = qk_chunk(n0 + u, (HP // 4) * t + u // 4, u % 4, c, bufs[u % 2],
                              m8 if c else None)
                if c == NC - 1:
                    if u == HP - 1:
                        m_scr[...] = m8
                    else:
                        ms.append(fin(m8))
                if ga >= LAG:
                    do_pv(ga - LAG)
            for gb in range(HP * NC - LAG, HP * NC):
                do_pv(gb)
            return carry
        lax.fori_loop(0, H // HP, hbody, 0)

    @pl.when(i == NQ)
    def _last_pv():
        m = fin(m_scr[...])
        finish((NI - 2) % (2 * H), acc_scr[...])
        acc = None
        for c in range(NC):
            acc = pv_chunk(H - 1, c, bufs[1], m, acc)
        finish((NI - 1) % (2 * H), acc)

    @pl.when(i >= 1)
    def _epilogue():
        tile = i - 1
        q0 = pl.multiple_of(tile * TQ, TQ)
        s0 = pl.multiple_of((tile % 2) * H, H)
        r64 = lax.broadcasted_iota(jnp.int32, (64, TE), 0)
        ones_rows = jnp.where(r64 == 0, 1.0, 0.0).astype(bf16)
        hs = []
        for e in range(NE):
            otn = otn_scr[pl.ds(s0, H), :, e * TE:(e + 1) * TE].reshape(H * DP, TE)
            attn = _dot(wot[...], otn)
            hs.append(x_v[:, pl.ds(q0 + e * TE, TE)].astype(f32) + attn)
        rs = []
        for e in range(NE):
            hn = jnp.concatenate([_ln_t(hs[e]).astype(bf16), ones_rows], axis=0)
            h1 = jnp.maximum(_dot(w1t[...], hn), 0.0)
            rs.append((h1 * h1).astype(bf16))
        b2t = jnp.concatenate([b2c[...]] * (TE // 128), axis=1)
        for e in range(NE):
            out = _dot(w2t_v[...], rs[e])
            c0 = pl.multiple_of(q0 + e * TE, 128)
            o_v[:, pl.ds(c0, TE)] = (hs[e] + b2t + out).astype(bf16)
            pltpu.make_async_copy(o_v.at[:, pl.ds(c0, TE)], o_hbm.at[:, pl.ds(c0, TE)], osem).start()

    @pl.when(i == NQ)
    def _drain():
        pltpu.make_async_copy(o_v, o_hbm, osem).wait()


@jax.jit
def pallas_sequential_preLN__mha_block__dense_activation_squared_relu__prompt_kernel(
    A_x: jax.Array,
    A_wqkv: jax.Array,
    A_wo: jax.Array,
    B_x: jax.Array,
    B_w1: jax.Array,
    B_b1: jax.Array,
    B_w2: jax.Array,
    B_b2: jax.Array,
):
    del B_x
    xt = A_x.reshape(S, D).T
    w2t = B_w2.T
    anyspec = pl.BlockSpec(memory_space=pl.ANY)
    out_t = pl.pallas_call(
        _kernel,
        grid=(NQ + 1,),
        in_specs=[anyspec] * 7,
        out_specs=anyspec,
        out_shape=jax.ShapeDtypeStruct((D, S), bf16),
        scratch_shapes=[
            pltpu.VMEM((D, S), bf16),
            pltpu.VMEM((D, 3 * D), bf16),
            pltpu.VMEM((D, D), bf16),
            pltpu.VMEM((D, F), bf16),
            pltpu.VMEM((D, F), bf16),
            pltpu.VMEM((3 * D, D), bf16),
            pltpu.VMEM((D, H * DP), bf16),
            pltpu.VMEM((F, 512), bf16),
            pltpu.VMEM((D, 128), f32),
            pltpu.VMEM((4, S, 128), bf16),
            pltpu.VMEM((H, DP, S), bf16),
            pltpu.VMEM((NI, QW, TQ), bf16),
            pltpu.VMEM((2, S, TQ), f32),
            pltpu.VMEM((2 * H, DP, TQ), bf16),
            pltpu.VMEM((D, S), bf16),
            pltpu.VMEM((D, 2 * TQ), bf16),
            pltpu.VMEM((8, TQ), f32),
            pltpu.VMEM((DP, TQ), f32),
            pltpu.VMEM((F,), bf16),
            pltpu.VMEM((D,), bf16),
            pltpu.SemaphoreType.DMA((8,)),
        ],
        compiler_params=pltpu.CompilerParams(
            dimension_semantics=("arbitrary",), vmem_limit_bytes=100 * 1024 * 1024,
            disable_bounds_checks=True, disable_semaphore_checks=True),
    )(xt, A_wqkv, A_wo, B_w1, w2t, B_b1, B_b2)
    return out_t.T.reshape(1, S, D)
```

```python
import jax
import jax.numpy as jnp
from jax import lax
import jax.experimental.pallas as pl
import jax.experimental.pallas.tpu as pltpu

S = 2048
D = 448
H = 16
DH = 28
DP = 32
G = 4 * DH
F = 1792
EPS = 1e-5
LOG2E = 1.4426950408889634
QSCALE = (DH ** -0.5) * LOG2E
f32 = jnp.float32
bf16 = jnp.bfloat16

TQ = 512
CK = 128
NE = 4
HP = 8
LAG = 2
FINISH_AT = 6
NQ = S // TQ
NC = S // CK
NI = NQ * H
TE = TQ // NE
QW = 48
QOFF = (0, 16, 48, 64)
WPIECES = ((0, 256), (256, 512), (512, 3 * D))


def _dot(a, b):
    return jnp.dot(a, b, preferred_element_type=f32)


def _colmean_fast(x):
    q = x.shape[0] // 4
    s = (x[0:q] + x[q:2 * q]) + (x[2 * q:3 * q] + x[3 * q:])
    return jnp.sum(s, axis=0, keepdims=True) * (1.0 / x.shape[0])


def _colmean(x):
    return jnp.sum(x, axis=0, keepdims=True) * (1.0 / x.shape[0])


def _ln_t(x, fast=False):
    mean = _colmean_fast if fast else _colmean
    xc = x - mean(x)
    v = mean(xc * xc)
    return xc * lax.rsqrt(v + EPS)


def _kernel(x_hbm, wqkv_hbm, wo_hbm, w1_hbm, w2t_hbm, b1_hbm, b2_hbm,
            o_hbm,
            x_v, wqkv_v, wo_v, w1_v, w2t_v, wall_t, wot, w1t, b2c,
            k_scr, vt_scr, qm_scr, s2_scr, otn_scr, o_v, xn_scr, m_scr, acc_scr,
            b1_v, b2_v, sems):
    i = pl.program_id(0)
    bufs = (s2_scr.at[0], s2_scr.at[1])
    osem = sems.at[7]

    def qk_chunk(a, g, j, c, s_scr, m):
        parts = []
        if QOFF[j]:
            parts.append(jnp.zeros((QOFF[j], TQ), bf16))
        parts.append(qm_scr[a])
        parts.append(jnp.zeros((128 - QW - QOFF[j], TQ), bf16))
        qm = jnp.concatenate(parts, axis=0)
        s = _dot(k_scr[g, c * CK:(c + 1) * CK, :], qm)
        s_scr[c * CK:(c + 1) * CK, :] = s
        sm = jnp.max(s.reshape(CK // 8, 8, TQ), axis=0)
        return sm if m is None else jnp.maximum(m, sm)

    def pv_chunk(h, c, s_scr, m, acc):
        p = jnp.exp2(s_scr[c * CK:(c + 1) * CK, :] - m).astype(bf16)
        o = _dot(vt_scr[h, :, c * CK:(c + 1) * CK], p)
        return o if acc is None else acc + o

    def fin(m8):
        return jnp.max(m8, axis=0, keepdims=True)

    def finish(slot, o):
        otn_scr[slot] = (o * (1.0 / o[DH:DH + 1, :])).astype(bf16)

    @pl.when(i == 0)
    def _prologue():
        def xcopy(lo, hi, sem):
            return pltpu.make_async_copy(x_hbm.at[:, lo:hi], x_v.at[:, lo:hi], sem)

        def wcopy(p, sem):
            lo, hi = WPIECES[p]
            return pltpu.make_async_copy(wqkv_hbm.at[:, lo:hi], wqkv_v.at[:, lo:hi], sem)

        th = TQ // 2
        stage = [
            [xcopy(0, th, sems.at[0])],
            [wcopy(0, sems.at[1])],
            [wcopy(1, sems.at[2]), xcopy(th, TQ, sems.at[2])],
            [wcopy(2, sems.at[3])],
            [xcopy(TQ, 2 * TQ, sems.at[4])],
            [xcopy(2 * TQ, S, sems.at[5])] + [
                pltpu.make_async_copy(src, dst, sems.at[5])
                for src, dst in ((wo_hbm, wo_v), (w1_hbm, w1_v), (b1_hbm, b1_v), (b2_hbm, b2_v))],
            [pltpu.make_async_copy(w2t_hbm, w2t_v, sems.at[6])],
        ]
        for st in stage:
            for cp in st:
                cp.start()

        def wait(k):
            for cp in stage[k]:
                cp.wait()

        def prep_w(p):
            lo, hi = WPIECES[p]
            wt = wqkv_v[:, lo:hi].T
            wall_t[lo:hi, :] = wt
            return wt

        r4 = lax.broadcasted_iota(jnp.int32, (DP - DH, TQ), 0)
        vpad = jnp.where(r4 == 0, 1.0, 0.0)
        kpad = jnp.zeros((128 - G, TQ), bf16)

        def proj(c, lo, hi, xn=None, t0=0, t1=TQ, w=None):
            if xn is None:
                xn = xn_scr[:, c * TQ + t0:c * TQ + t1]
            r = _dot(wall_t[lo:hi, :] if w is None else w, xn)
            roww = lax.broadcasted_iota(jnp.int32, (QW, t1 - t0), 0)
            for g in range(4):
                if lo <= G * g < hi:
                    for j in range(4):
                        o = G * g + QOFF[j] - lo
                        qw = r[o:o + QW, :] * QSCALE
                        b = DH * j - QOFF[j]
                        msk = (roww >= b) & (roww < b + DH)
                        qm_scr[c * H + 4 * g + j, :, t0:t1] = jnp.where(msk, qw, 0.0).astype(bf16)
            for g in range(4):
                if lo <= D + G * g < hi:
                    o = D + G * g - lo
                    kg = jnp.concatenate([r[o:o + G, :].astype(bf16), kpad], axis=0)
                    k_scr[g, c * TQ:(c + 1) * TQ, :] = kg.T
            for h in range(H):
                if lo <= 2 * D + DH * h < hi:
                    o = 2 * D + DH * h - lo
                    vt = jnp.concatenate([r[o:o + DH, :], vpad], axis=0)
                    vt_scr[h, :, c * TQ:(c + 1) * TQ] = vt.astype(bf16)

        def ln_tile(c0):
            return _ln_t(x_v[:, c0:c0 + 128].astype(f32), c0 < th).astype(bf16)

        def ln_store(lo, hi):
            for c0 in range(lo, hi, 128):
                xn_scr[:, c0:c0 + 128] = ln_tile(c0)

        bufs[1][...] = jnp.zeros((S, TQ), f32)
        m_scr[...] = jnp.zeros((8, TQ), f32)
        acc_scr[...] = jnp.ones((DP, TQ), f32)

        wait(0)
        ln_store(0, th)
        wait(1)
        wt = prep_w(0)
        proj(0, 0, G, None, 0, th, wt[0:G])
        wait(2)
        proj(0, G, 2 * G, None, 0, th)
        prep_w(1)
        proj(0, 2 * G, D, None, 0, th)
        ln_store(th, TQ)
        proj(0, 0, 3 * G, None, th, TQ)
        wait(3)
        proj(0, 3 * G, D, None, th, TQ)
        prep_w(2)
        proj(0, 2 * D, 3 * D)
        wait(4)
        proj(0, D, 2 * D)
        ln_store(TQ, 2 * TQ)
        proj(1, D, 2 * D)
        proj(1, 0, D)
        wait(5)
        proj(1, 2 * D, 3 * D)
        for c in range(2, NQ):
            xn = jnp.concatenate([ln_tile(c0) for c0 in range(c * TQ, (c + 1) * TQ, 128)], axis=1)
            proj(c, 0, 3 * D, xn)

        wo32 = wo_v[...].astype(f32)
        zpad = jnp.zeros((DP - DH, D), f32)
        blks = []
        for h in range(H):
            blks.append(wo32[DH * h:DH * (h + 1), :])
            blks.append(zpad)
        wot[...] = jnp.concatenate(blks, axis=0).astype(bf16).T
        r64 = lax.broadcasted_iota(jnp.int32, (64, F), 0)
        b1row = b1_v[...].reshape(1, F).astype(f32)
        extra = jnp.where(r64 == 0, b1row, 0.0).astype(bf16)
        w1t[...] = jnp.concatenate([w1_v[...], extra], axis=0).T
        b2row = b2_v[...].reshape(1, D).astype(f32)
        b2c[...] = jnp.broadcast_to(b2row, (128, D)).T
        wait(6)

    @pl.when(i < NQ)
    def _attention():
        def hbody(t, carry):
            n0 = i * H + HP * t
            ms = [fin(m_scr[...])]
            accs = {}
            m8 = None

            def do_pv(gb):
                u, c = divmod(gb, NC)
                accs[u] = pv_chunk((n0 + u - 1) & (H - 1), c, bufs[(u + 1) % 2], ms[u], accs.get(u))
                if c == FINISH_AT:
                    finish((n0 + u - 2) & (2 * H - 1), acc_scr[...])
                if c == NC - 1:
                    acc_scr[...] = accs[u]

            for ga in range(HP * NC):
                u, c = divmod(ga, NC)
                m8 = qk_chunk(n0 + u, (HP // 4) * t + u // 4, u % 4, c, bufs[u % 2],
                              m8 if c else None)
                if c == NC - 1:
                    if u == HP - 1:
                        m_scr[...] = m8
                    else:
                        ms.append(fin(m8))
                if ga >= LAG:
                    do_pv(ga - LAG)
            for gb in range(HP * NC - LAG, HP * NC):
                do_pv(gb)
            return carry
        lax.fori_loop(0, H // HP, hbody, 0)

    @pl.when(i == NQ)
    def _last_pv():
        m = fin(m_scr[...])
        finish((NI - 2) % (2 * H), acc_scr[...])
        acc = None
        for c in range(NC):
            acc = pv_chunk(H - 1, c, bufs[1], m, acc)
        finish((NI - 1) % (2 * H), acc)

    @pl.when(i >= 1)
    def _epilogue():
        tile = i - 1
        q0 = pl.multiple_of(tile * TQ, TQ)
        s0 = pl.multiple_of((tile % 2) * H, H)
        r64 = lax.broadcasted_iota(jnp.int32, (64, TE), 0)
        ones_rows = jnp.where(r64 == 0, 1.0, 0.0).astype(bf16)
        hs = []
        for e in range(NE):
            otn = otn_scr[pl.ds(s0, H), :, e * TE:(e + 1) * TE].reshape(H * DP, TE)
            attn = _dot(wot[...], otn)
            hs.append(x_v[:, pl.ds(q0 + e * TE, TE)].astype(f32) + attn)
        rs = []
        for e in range(NE):
            hn = jnp.concatenate([_ln_t(hs[e]).astype(bf16), ones_rows], axis=0)
            h1 = jnp.maximum(_dot(w1t[...], hn), 0.0)
            rs.append((h1 * h1).astype(bf16))
        b2t = jnp.concatenate([b2c[...]] * (TE // 128), axis=1)
        for e in range(NE):
            out = _dot(w2t_v[...], rs[e])
            c0 = pl.multiple_of(q0 + e * TE, 128)
            o_v[:, pl.ds(c0, TE)] = (hs[e] + b2t + out).astype(bf16)
            pltpu.make_async_copy(o_v.at[:, pl.ds(c0, TE)], o_hbm.at[:, pl.ds(c0, TE)], osem).start()

    @pl.when(i == NQ)
    def _drain():
        pltpu.make_async_copy(o_v, o_hbm, osem).wait()


@jax.jit
def pallas_sequential_preLN__mha_block__dense_activation_squared_relu__prompt_kernel(
    A_x: jax.Array,
    A_wqkv: jax.Array,
    A_wo: jax.Array,
    B_x: jax.Array,
    B_w1: jax.Array,
    B_b1: jax.Array,
    B_w2: jax.Array,
    B_b2: jax.Array,
):
    del B_x
    xt = A_x.reshape(S, D).T
    w2t = B_w2.T
    anyspec = pl.BlockSpec(memory_space=pl.ANY)
    out_t = pl.pallas_call(
        _kernel,
        grid=(NQ + 1,),
        in_specs=[anyspec] * 7,
        out_specs=anyspec,
        out_shape=jax.ShapeDtypeStruct((D, S), bf16),
        scratch_shapes=[
            pltpu.VMEM((D, S), bf16),
            pltpu.VMEM((D, 3 * D), bf16),
            pltpu.VMEM((D, D), bf16),
            pltpu.VMEM((D, F), bf16),
            pltpu.VMEM((D, F), bf16),
            pltpu.VMEM((3 * D, D), bf16),
            pltpu.VMEM((D, H * DP), bf16),
            pltpu.VMEM((F, 512), bf16),
            pltpu.VMEM((D, 128), f32),
            pltpu.VMEM((4, S, 128), bf16),
            pltpu.VMEM((H, DP, S), bf16),
            pltpu.VMEM((NI, QW, TQ), bf16),
            pltpu.VMEM((2, S, TQ), f32),
            pltpu.VMEM((2 * H, DP, TQ), bf16),
            pltpu.VMEM((D, S), bf16),
            pltpu.VMEM((D, 2 * TQ), bf16),
            pltpu.VMEM((8, TQ), f32),
            pltpu.VMEM((DP, TQ), f32),
            pltpu.VMEM((F,), bf16),
            pltpu.VMEM((D,), bf16),
            pltpu.SemaphoreType.DMA((8,)),
        ],
        compiler_params=pltpu.CompilerParams(
            dimension_semantics=("arbitrary",), vmem_limit_bytes=100 * 1024 * 1024,
            disable_bounds_checks=True, disable_semaphore_checks=True),
    )(xt, A_wqkv, A_wo, B_w1, w2t, B_b1, B_b2)
    return out_t.T.reshape(1, S, D)
```

```python
import jax
import jax.numpy as jnp
from jax import lax
import jax.experimental.pallas as pl
import jax.experimental.pallas.tpu as pltpu

S = 2048
D = 448
H = 16
DH = 28
DP = 32
G = 4 * DH
F = 1792
EPS = 1e-5
LOG2E = 1.4426950408889634
QSCALE = (DH ** -0.5) * LOG2E
f32 = jnp.float32
bf16 = jnp.bfloat16

TQ = 512
CK = 128
NE = 4
HP = 8
LAG = 3
FINISH_AT = 2
NQ = S // TQ
NC = S // CK
NI = NQ * H
TE = TQ // NE
QW = 48
QOFF = (0, 16, 48, 64)
WPIECES = ((0, 256), (256, 512), (512, 3 * D))


def _dot(a, b):
    return jnp.dot(a, b, preferred_element_type=f32)


def _colmean_fast(x):
    q = x.shape[0] // 4
    s = (x[0:q] + x[q:2 * q]) + (x[2 * q:3 * q] + x[3 * q:])
    return jnp.sum(s, axis=0, keepdims=True) * (1.0 / x.shape[0])


def _colmean(x):
    return jnp.sum(x, axis=0, keepdims=True) * (1.0 / x.shape[0])


def _ln_t(x, fast=False):
    mean = _colmean_fast if fast else _colmean
    xc = x - mean(x)
    v = mean(xc * xc)
    return xc * lax.rsqrt(v + EPS)


def _kernel(x_hbm, wqkv_hbm, wo_hbm, w1_hbm, w2t_hbm, b1_hbm, b2_hbm,
            o_hbm,
            x_v, wqkv_v, wo_v, w1_v, w2t_v, wall_t, wot, w1t, b2c,
            k_scr, vt_scr, qm_scr, s_scr, otn_scr, o_v, xn_scr, m_scr, mp_scr, acc2_scr,
            b1_v, b2_v, sems):
    i = pl.program_id(0)
    acc_scr = acc2_scr.at[0]
    done_scr = acc2_scr.at[1]
    osem = sems.at[7]

    def qk_chunk(a, g, j, c, m):
        parts = []
        if QOFF[j]:
            parts.append(jnp.zeros((QOFF[j], TQ), bf16))
        parts.append(qm_scr[a])
        parts.append(jnp.zeros((128 - QW - QOFF[j], TQ), bf16))
        qm = jnp.concatenate(parts, axis=0)
        s = _dot(k_scr[g, c * CK:(c + 1) * CK, :], qm)
        s_scr[c * CK:(c + 1) * CK, :] = s
        sm = jnp.max(s.reshape(CK // 8, 8, TQ), axis=0)
        return sm if m is None else jnp.maximum(m, sm)

    def pv_chunk(h, c, m_old, m, acc):
        if acc is not None:
            acc = acc * jnp.exp2(m_old - m)
        p = jnp.exp2(s_scr[c * CK:(c + 1) * CK, :] - m).astype(bf16)
        o = _dot(vt_scr[h, :, c * CK:(c + 1) * CK], p)
        return o if acc is None else acc + o

    def fin(m8):
        return jnp.max(m8, axis=0, keepdims=True)

    def finish(slot, o):
        otn_scr[slot] = (o * (1.0 / o[DH:DH + 1, :])).astype(bf16)

    @pl.when(i == 0)
    def _prologue():
        def xcopy(lo, hi, sem):
            return pltpu.make_async_copy(x_hbm.at[:, lo:hi], x_v.at[:, lo:hi], sem)

        def wcopy(p, sem):
            lo, hi = WPIECES[p]
            return pltpu.make_async_copy(wqkv_hbm.at[:, lo:hi], wqkv_v.at[:, lo:hi], sem)

        th = TQ // 2
        stage = [
            [xcopy(0, th, sems.at[0])],
            [wcopy(0, sems.at[1])],
            [wcopy(1, sems.at[2]), xcopy(th, TQ, sems.at[2])],
            [wcopy(2, sems.at[3])],
            [xcopy(TQ, 2 * TQ, sems.at[4])],
            [xcopy(2 * TQ, S, sems.at[5])] + [
                pltpu.make_async_copy(src, dst, sems.at[5])
                for src, dst in ((wo_hbm, wo_v), (w1_hbm, w1_v), (b1_hbm, b1_v), (b2_hbm, b2_v))],
            [pltpu.make_async_copy(w2t_hbm, w2t_v, sems.at[6])],
        ]
        for st in stage:
            for cp in st:
                cp.start()

        def wait(k):
            for cp in stage[k]:
                cp.wait()

        def prep_w(p):
            lo, hi = WPIECES[p]
            wt = wqkv_v[:, lo:hi].T
            wall_t[lo:hi, :] = wt
            return wt

        r4 = lax.broadcasted_iota(jnp.int32, (DP - DH, TQ), 0)
        vpad = jnp.where(r4 == 0, 1.0, 0.0)
        kpad = jnp.zeros((128 - G, TQ), bf16)

        def proj(c, lo, hi, xn=None, t0=0, t1=TQ, w=None):
            if xn is None:
                xn = xn_scr[:, c * TQ + t0:c * TQ + t1]
            r = _dot(wall_t[lo:hi, :] if w is None else w, xn)
            roww = lax.broadcasted_iota(jnp.int32, (QW, t1 - t0), 0)
            for g in range(4):
                if lo <= G * g < hi:
                    for j in range(4):
                        o = G * g + QOFF[j] - lo
                        qw = r[o:o + QW, :] * QSCALE
                        b = DH * j - QOFF[j]
                        msk = (roww >= b) & (roww < b + DH)
                        qm_scr[c * H + 4 * g + j, :, t0:t1] = jnp.where(msk, qw, 0.0).astype(bf16)
            for g in range(4):
                if lo <= D + G * g < hi:
                    o = D + G * g - lo
                    kg = jnp.concatenate([r[o:o + G, :].astype(bf16), kpad], axis=0)
                    k_scr[g, c * TQ:(c + 1) * TQ, :] = kg.T
            for h in range(H):
                if lo <= 2 * D + DH * h < hi:
                    o = 2 * D + DH * h - lo
                    vt = jnp.concatenate([r[o:o + DH, :], vpad], axis=0)
                    vt_scr[h, :, c * TQ:(c + 1) * TQ] = vt.astype(bf16)

        def ln_tile(c0):
            return _ln_t(x_v[:, c0:c0 + 128].astype(f32), c0 < th).astype(bf16)

        def ln_store(lo, hi):
            for c0 in range(lo, hi, 128):
                xn_scr[:, c0:c0 + 128] = ln_tile(c0)

        s_scr[S - CK:, :] = jnp.zeros((CK, TQ), f32)
        mp_scr[...] = jnp.zeros((8, TQ), f32)
        m_scr[...] = jnp.zeros((8, TQ), f32)
        acc_scr[...] = jnp.ones((DP, TQ), f32)

        wait(0)
        ln_store(0, th)
        wait(1)
        wt = prep_w(0)
        proj(0, 0, G, None, 0, th, wt[0:G])
        wait(2)
        proj(0, G, 2 * G, None, 0, th)
        prep_w(1)
        proj(0, 2 * G, D, None, 0, th)
        ln_store(th, TQ)
        proj(0, 0, 3 * G, None, th, TQ)
        wait(3)
        proj(0, 3 * G, D, None, th, TQ)
        prep_w(2)
        proj(0, 2 * D, 3 * D)
        wait(4)
        proj(0, D, 2 * D)
        ln_store(TQ, 2 * TQ)
        proj(1, D, 2 * D)
        proj(1, 0, D)
        wait(5)
        proj(1, 2 * D, 3 * D)
        for c in range(2, NQ):
            xn = jnp.concatenate([ln_tile(c0) for c0 in range(c * TQ, (c + 1) * TQ, 128)], axis=1)
            proj(c, 0, 3 * D, xn)

        wo32 = wo_v[...].astype(f32)
        zpad = jnp.zeros((DP - DH, D), f32)
        blks = []
        for h in range(H):
            blks.append(wo32[DH * h:DH * (h + 1), :])
            blks.append(zpad)
        wot[...] = jnp.concatenate(blks, axis=0).astype(bf16).T
        r64 = lax.broadcasted_iota(jnp.int32, (64, F), 0)
        b1row = b1_v[...].reshape(1, F).astype(f32)
        extra = jnp.where(r64 == 0, b1row, 0.0).astype(bf16)
        w1t[...] = jnp.concatenate([w1_v[...], extra], axis=0).T
        b2row = b2_v[...].reshape(1, D).astype(f32)
        b2c[...] = jnp.broadcast_to(b2row, (128, D)).T
        wait(6)

    @pl.when(i < NQ)
    def _attention():
        def hbody(t, carry):
            n0 = i * H + HP * t
            mrun = {-1: fin(m_scr[...]), -2: mp_scr[0:1, :]}
            accs = {-1: acc_scr[...]}
            m8 = None

            def do_pv(gb):
                u, c = divmod(gb, NC)
                accs[u] = pv_chunk((n0 + u) & (H - 1), c, mrun[gb - 1], mrun[gb], accs.get(u))
                if c == FINISH_AT:
                    finish((n0 + u - 1) & (2 * H - 1), done_scr[...])
                if c == NC - 1:
                    done_scr[...] = accs[u]

            last = HP * NC - 1
            for ga in range(HP * NC):
                u, c = divmod(ga, NC)
                m8 = qk_chunk(n0 + u, (HP // 4) * t + u // 4, u % 4, c, m8 if c else None)
                if ga == last:
                    m_scr[...] = m8
                else:
                    mrun[ga] = fin(m8)
                if ga >= LAG - 1:
                    do_pv(ga - LAG)
            for gb in range(last + 1 - LAG, last):
                do_pv(gb)
            acc_scr[...] = accs[HP - 1]
            mp_scr[0:1, :] = mrun[last - 1]
            return carry
        lax.fori_loop(0, H // HP, hbody, 0)

    @pl.when(i == NQ)
    def _last_pv():
        acc = pv_chunk(H - 1, NC - 1, mp_scr[0:1, :], fin(m_scr[...]), acc_scr[...])
        finish((NI - 1) % (2 * H), acc)

    @pl.when(i >= 1)
    def _epilogue():
        tile = i - 1
        q0 = pl.multiple_of(tile * TQ, TQ)
        s0 = pl.multiple_of((tile % 2) * H, H)
        r64 = lax.broadcasted_iota(jnp.int32, (64, TE), 0)
        ones_rows = jnp.where(r64 == 0, 1.0, 0.0).astype(bf16)
        hs = []
        for e in range(NE):
            otn = otn_scr[pl.ds(s0, H), :, e * TE:(e + 1) * TE].reshape(H * DP, TE)
            attn = _dot(wot[...], otn)
            hs.append(x_v[:, pl.ds(q0 + e * TE, TE)].astype(f32) + attn)
        rs = []
        for e in range(NE):
            hn = jnp.concatenate([_ln_t(hs[e]).astype(bf16), ones_rows], axis=0)
            h1 = jnp.maximum(_dot(w1t[...], hn), 0.0)
            rs.append((h1 * h1).astype(bf16))
        b2t = jnp.concatenate([b2c[...]] * (TE // 128), axis=1)
        for e in range(NE):
            out = _dot(w2t_v[...], rs[e])
            c0 = pl.multiple_of(q0 + e * TE, 128)
            o_v[:, pl.ds(c0, TE)] = (hs[e] + b2t + out).astype(bf16)
            pltpu.make_async_copy(o_v.at[:, pl.ds(c0, TE)], o_hbm.at[:, pl.ds(c0, TE)], osem).start()

    @pl.when(i == NQ)
    def _drain():
        pltpu.make_async_copy(o_v, o_hbm, osem).wait()


@jax.jit
def pallas_sequential_preLN__mha_block__dense_activation_squared_relu__prompt_kernel(
    A_x: jax.Array,
    A_wqkv: jax.Array,
    A_wo: jax.Array,
    B_x: jax.Array,
    B_w1: jax.Array,
    B_b1: jax.Array,
    B_w2: jax.Array,
    B_b2: jax.Array,
):
    del B_x
    xt = A_x.reshape(S, D).T
    w2t = B_w2.T
    anyspec = pl.BlockSpec(memory_space=pl.ANY)
    out_t = pl.pallas_call(
        _kernel,
        grid=(NQ + 1,),
        in_specs=[anyspec] * 7,
        out_specs=anyspec,
        out_shape=jax.ShapeDtypeStruct((D, S), bf16),
        scratch_shapes=[
            pltpu.VMEM((D, S), bf16),
            pltpu.VMEM((D, 3 * D), bf16),
            pltpu.VMEM((D, D), bf16),
            pltpu.VMEM((D, F), bf16),
            pltpu.VMEM((D, F), bf16),
            pltpu.VMEM((3 * D, D), bf16),
            pltpu.VMEM((D, H * DP), bf16),
            pltpu.VMEM((F, 512), bf16),
            pltpu.VMEM((D, 128), f32),
            pltpu.VMEM((4, S, 128), bf16),
            pltpu.VMEM((H, DP, S), bf16),
            pltpu.VMEM((NI, QW, TQ), bf16),
            pltpu.VMEM((S, TQ), f32),
            pltpu.VMEM((2 * H, DP, TQ), bf16),
            pltpu.VMEM((D, S), bf16),
            pltpu.VMEM((D, 2 * TQ), bf16),
            pltpu.VMEM((8, TQ), f32),
            pltpu.VMEM((8, TQ), f32),
            pltpu.VMEM((2, DP, TQ), f32),
            pltpu.VMEM((F,), bf16),
            pltpu.VMEM((D,), bf16),
            pltpu.SemaphoreType.DMA((8,)),
        ],
        compiler_params=pltpu.CompilerParams(
            dimension_semantics=("arbitrary",), vmem_limit_bytes=100 * 1024 * 1024,
            disable_bounds_checks=True, disable_semaphore_checks=True),
    )(xt, A_wqkv, A_wo, B_w1, w2t, B_b1, B_b2)
    return out_t.T.reshape(1, S, D)
```

```python
import jax
import jax.numpy as jnp
from jax import lax
import jax.experimental.pallas as pl
import jax.experimental.pallas.tpu as pltpu

S = 2048
D = 448
H = 16
DH = 28
DP = 32
G = 4 * DH
F = 1792
EPS = 1e-5
LOG2E = 1.4426950408889634
QSCALE = (DH ** -0.5) * LOG2E
f32 = jnp.float32
bf16 = jnp.bfloat16

TP = 512
NP = S // TP
CK = 128
NC = S // CK
NT = 2
NB = S // (128 * NT)
LAG = 2
NSLOT = 8
FINISH_AT = 2
WO_AT = 6
QW = 48
QOFF = (0, 16, 48, 64)
WPIECES = ((0, 256), (256, 512), (512, 3 * D))


def _dot(a, b):
    return jnp.dot(a, b, preferred_element_type=f32)


def _colmean_fast(x):
    q = x.shape[0] // 4
    s = (x[0:q] + x[q:2 * q]) + (x[2 * q:3 * q] + x[3 * q:])
    return jnp.sum(s, axis=0, keepdims=True) * (1.0 / x.shape[0])


def _colmean(x):
    return jnp.sum(x, axis=0, keepdims=True) * (1.0 / x.shape[0])


def _ln_t(x, fast=False):
    mean = _colmean_fast if fast else _colmean
    xc = x - mean(x)
    v = mean(xc * xc)
    return xc * lax.rsqrt(v + EPS)


def _kernel(x_hbm, wqkv_hbm, wo_hbm, w1_hbm, w2t_hbm, b1_hbm, b2_hbm,
            o_hbm,
            x_v, wqkv_v, wo_v, w1_v, w2t_v, wall_t, wot, w1t, b2c,
            k_scr, vt_scr, qm_scr, s_scr, otn_scr, o_v, xn_scr, done_scr,
            b1_v, b2_v, sems):
    i = pl.program_id(0)
    osem = sems.at[7]

    @pl.when(i == 0)
    def _prologue():
        def xcopy(lo, hi, sem):
            return pltpu.make_async_copy(x_hbm.at[:, lo:hi], x_v.at[:, lo:hi], sem)

        def wcopy(p, sem):
            lo, hi = WPIECES[p]
            return pltpu.make_async_copy(wqkv_hbm.at[:, lo:hi], wqkv_v.at[:, lo:hi], sem)

        th = TP // 2
        stage = [
            [xcopy(0, th, sems.at[0])],
            [wcopy(0, sems.at[1])],
            [wcopy(1, sems.at[2]), xcopy(th, TP, sems.at[2])],
            [wcopy(2, sems.at[3])],
            [xcopy(TP, 2 * TP, sems.at[4])],
            [xcopy(2 * TP, S, sems.at[5])] + [
                pltpu.make_async_copy(src, dst, sems.at[5])
                for src, dst in ((wo_hbm, wo_v), (w1_hbm, w1_v), (b1_hbm, b1_v), (b2_hbm, b2_v))],
            [pltpu.make_async_copy(w2t_hbm, w2t_v, sems.at[6])],
        ]
        for st in stage:
            for cp in st:
                cp.start()

        def wait(k):
            for cp in stage[k]:
                cp.wait()

        def prep_w(p):
            lo, hi = WPIECES[p]
            wt = wqkv_v[:, lo:hi].T
            wall_t[lo:hi, :] = wt
            return wt

        r4 = lax.broadcasted_iota(jnp.int32, (DP - DH, TP), 0)
        vpad = jnp.where(r4 == 0, 1.0, 0.0)
        kpad = jnp.zeros((128 - G, TP), bf16)

        def proj(c, lo, hi, xn=None, t0=0, t1=TP, w=None):
            if xn is None:
                xn = xn_scr[:, c * TP + t0:c * TP + t1]
            r = _dot(wall_t[lo:hi, :] if w is None else w, xn)
            roww = lax.broadcasted_iota(jnp.int32, (QW, t1 - t0), 0)
            for g in range(4):
                if lo <= G * g < hi:
                    for j in range(4):
                        o = G * g + QOFF[j] - lo
                        b = DH * j - QOFF[j]
                        msk = (roww >= b) & (roww < b + DH)
                        qw = jnp.where(msk, r[o:o + QW, :] * QSCALE, 0.0)
                        for l in range((t1 - t0) // 128):
                            qm_scr[(c * TP + t0) // 128 + l, 4 * g + j] = (
                                qw[:, l * 128:(l + 1) * 128].astype(bf16))
            for g in range(4):
                if lo <= D + G * g < hi:
                    o = D + G * g - lo
                    kg = jnp.concatenate([r[o:o + G, :].astype(bf16), kpad], axis=0)
                    k_scr[g, c * TP:(c + 1) * TP, :] = kg.T
            for h in range(H):
                if lo <= 2 * D + DH * h < hi:
                    o = 2 * D + DH * h - lo
                    vt = jnp.concatenate([r[o:o + DH, :], vpad], axis=0)
                    for l in range(TP // 128):
                        vt_scr[c * TP // 128 + l, h] = vt[:, l * 128:(l + 1) * 128].astype(bf16)

        def ln_tile(c0):
            return _ln_t(x_v[:, c0:c0 + 128].astype(f32), c0 < th).astype(bf16)

        def ln_store(lo, hi):
            for c0 in range(lo, hi, 128):
                xn_scr[:, c0:c0 + 128] = ln_tile(c0)

        s_scr[0:8, :] = jnp.zeros((8, 512), f32)
        done_scr[0:8, :] = jnp.zeros((8, 512), f32)
        otn_scr[0, 0:16, :] = jnp.zeros((16, 128), bf16)

        wait(0)
        ln_store(0, th)
        wait(1)
        wt = prep_w(0)
        proj(0, 0, G, None, 0, th, wt[0:G])
        wait(2)
        proj(0, G, 2 * G, None, 0, th)
        prep_w(1)
        proj(0, 2 * G, D, None, 0, th)
        ln_store(th, TP)
        proj(0, 0, 3 * G, None, th, TP)
        wait(3)
        proj(0, 3 * G, D, None, th, TP)
        prep_w(2)
        proj(0, 2 * D, 3 * D)
        wait(4)
        proj(0, D, 2 * D)
        ln_store(TP, 2 * TP)
        proj(1, D, 2 * D)
        proj(1, 0, D)
        wait(5)
        proj(1, 2 * D, 3 * D)
        for c in range(2, NP):
            xn = jnp.concatenate([ln_tile(c0) for c0 in range(c * TP, (c + 1) * TP, 128)], axis=1)
            proj(c, 0, 3 * D, xn)

        wo32 = wo_v[...].astype(f32)
        zpad = jnp.zeros((DP - DH, D), f32)
        blks = []
        for h in range(H):
            blks.append(wo32[DH * h:DH * (h + 1), :])
            blks.append(zpad)
        wot[...] = jnp.concatenate(blks, axis=0).astype(bf16).T
        r64 = lax.broadcasted_iota(jnp.int32, (64, F), 0)
        b1row = b1_v[...].reshape(1, F).astype(f32)
        extra = jnp.where(r64 == 0, b1row, 0.0).astype(bf16)
        w1t[...] = jnp.concatenate([w1_v[...], extra], axis=0).T
        b2row = b2_v[...].reshape(1, D).astype(f32)
        b2c[...] = jnp.broadcast_to(b2row, (128, D)).T
        wait(6)

    q0s = [pl.multiple_of((i * NT + e) * 128, 128) for e in range(NT)]

    def qk_chunk(e, g, ga, m):
        c = ga % NC
        cols = []
        for j in range(4):
            parts = []
            if QOFF[j]:
                parts.append(jnp.zeros((QOFF[j], 128), bf16))
            parts.append(qm_scr[i * NT + e, 4 * g + j])
            parts.append(jnp.zeros((128 - QW - QOFF[j], 128), bf16))
            cols.append(jnp.concatenate(parts, axis=0))
        s = _dot(k_scr[g, c * CK:(c + 1) * CK, :], jnp.concatenate(cols, axis=1))
        sl = ga % NSLOT
        s_scr[sl * CK:(sl + 1) * CK, :] = s
        sm = jnp.max(s.reshape(CK // 8, 8, 512), axis=0)
        return sm if m is None else jnp.maximum(m, sm)

    def pv_chunk(g, gb, m_old, m, acc):
        c = gb % NC
        sl = gb % NSLOT
        if acc is not None:
            acc = acc * jnp.exp2(m_old - m)
        p = jnp.exp2(s_scr[sl * CK:(sl + 1) * CK, :] - m)
        o = jnp.concatenate(
            [_dot(vt_scr[c, 4 * g + j], p[:, j * 128:(j + 1) * 128].astype(bf16))
             for j in range(4)], axis=1)
        return o if acc is None else acc + o

    def finish(u, o):
        e, g = divmod(u, 4)
        on = (o * (1.0 / o[DH:DH + 1, :])).astype(bf16)
        for j in range(4):
            otn_scr[e, (4 * g + j) * DP:(4 * g + j + 1) * DP, :] = on[:, j * 128:(j + 1) * 128]

    r64 = lax.broadcasted_iota(jnp.int32, (64, 128), 0)
    ones_rows = jnp.where(r64 == 0, 1.0, 0.0).astype(bf16)
    hs = {}
    hns = {}
    rs = {}

    def st_wo(e):
        attn = _dot(wot[...], otn_scr[e])
        hs[e] = x_v[:, pl.ds(q0s[e], 128)].astype(f32) + attn
        hns[e] = jnp.concatenate([_ln_t(hs[e]).astype(bf16), ones_rows], axis=0)

    def st_f1(e, lo=0, hi=F):
        h1 = jnp.maximum(_dot(w1t[lo:hi, :], hns[e]), 0.0)
        rs.setdefault(e, []).append((h1 * h1).astype(bf16))

    def st_f2(e):
        out = _dot(w2t_v[...], jnp.concatenate(rs[e], axis=0))
        o_v[:, pl.ds(q0s[e], 128)] = (hs[e] + b2c[...] + out).astype(bf16)
        pltpu.make_async_copy(o_v.at[:, pl.ds(q0s[e], 128)], o_hbm.at[:, pl.ds(q0s[e], 128)],
                              osem).start()

    mrun = {}
    accs = {}
    NU = 4 * NT
    NG = NU * NC

    def do_pv(gb):
        u, c = divmod(gb, NC)
        accs[u] = pv_chunk(u % 4, gb, mrun.get(gb - 1), mrun[gb], accs.get(u))
        if c == FINISH_AT and u >= 1:
            finish(u - 1, done_scr[...])
        if c == NC - 1 and u < NU - 1:
            done_scr[...] = accs[u]
        if c == WO_AT and u % 4 == 0 and u >= 4:
            st_wo(u // 4 - 1)

    m8 = None
    for ga in range(NG):
        u, c = divmod(ga, NC)
        m8 = qk_chunk(u // 4, u % 4, ga, m8 if c else None)
        mrun[ga] = jnp.max(m8, axis=0, keepdims=True)
        if ga >= LAG:
            do_pv(ga - LAG)
    npc = LAG + 2
    bounds = [(F // 128 * k // npc) * 128 for k in range(npc + 1)]
    for k in range(npc):
        st_f1(0, bounds[k], bounds[k + 1])
        if k < LAG:
            do_pv(NG - LAG + k)
        if k == LAG - 1:
            finish(NU - 1, accs[NU - 1])
        if k == LAG:
            st_wo(NT - 1)
    for e in range(1, NT - 1):
        st_f1(e)
    for e in range(NT - 1):
        st_f2(e)
    st_f1(NT - 1)
    st_f2(NT - 1)

    @pl.when(i == NB - 1)
    def _drain():
        pltpu.make_async_copy(o_v, o_hbm, osem).wait()


@jax.jit
def pallas_sequential_preLN__mha_block__dense_activation_squared_relu__prompt_kernel(
    A_x: jax.Array,
    A_wqkv: jax.Array,
    A_wo: jax.Array,
    B_x: jax.Array,
    B_w1: jax.Array,
    B_b1: jax.Array,
    B_w2: jax.Array,
    B_b2: jax.Array,
):
    del B_x
    xt = A_x.reshape(S, D).T
    w2t = B_w2.T
    anyspec = pl.BlockSpec(memory_space=pl.ANY)
    out_t = pl.pallas_call(
        _kernel,
        grid=(NB,),
        in_specs=[anyspec] * 7,
        out_specs=anyspec,
        out_shape=jax.ShapeDtypeStruct((D, S), bf16),
        scratch_shapes=[
            pltpu.VMEM((D, S), bf16),
            pltpu.VMEM((D, 3 * D), bf16),
            pltpu.VMEM((D, D), bf16),
            pltpu.VMEM((D, F), bf16),
            pltpu.VMEM((D, F), bf16),
            pltpu.VMEM((3 * D, D), bf16),
            pltpu.VMEM((D, H * DP), bf16),
            pltpu.VMEM((F, 512), bf16),
            pltpu.VMEM((D, 128), f32),
            pltpu.VMEM((4, S, 128), bf16),
            pltpu.VMEM((NC, H, DP, 128), bf16),
            pltpu.VMEM((S // 128, H, QW, 128), bf16),
            pltpu.VMEM((NSLOT * CK, 512), f32),
            pltpu.VMEM((NT, H * DP, 128), bf16),
            pltpu.VMEM((D, S), bf16),
            pltpu.VMEM((D, 2 * TP), bf16),
            pltpu.VMEM((DP, 512), f32),
            pltpu.VMEM((F,), bf16),
            pltpu.VMEM((D,), bf16),
            pltpu.SemaphoreType.DMA((8,)),
        ],
        compiler_params=pltpu.CompilerParams(
            dimension_semantics=("arbitrary",), vmem_limit_bytes=100 * 1024 * 1024,
            disable_bounds_checks=True, disable_semaphore_checks=True),
    )(xt, A_wqkv, A_wo, B_w1, w2t, B_b1, B_b2)
    return out_t.T.reshape(1, S, D)
```

```python
import jax
import jax.numpy as jnp
from jax import lax
import jax.experimental.pallas as pl
import jax.experimental.pallas.tpu as pltpu

S = 2048
D = 448
H = 16
DH = 28
DP = 32
G = 4 * DH
F = 1792
EPS = 1e-5
LOG2E = 1.4426950408889634
QSCALE = (DH ** -0.5) * LOG2E
f32 = jnp.float32
bf16 = jnp.bfloat16

TP = 512
NP = S // TP
CK = 128
NC = S // CK
NT = 2
NB = S // (128 * NT)
LAG = 2
NSLOT = 8
FINISH_AT = 2
WO_AT = 6
QW = 48
QOFF = (0, 16, 48, 64)
WPIECES = ((0, 256), (256, 512), (512, 3 * D))


def _dot(a, b):
    return jnp.dot(a, b, preferred_element_type=f32)


def _colmean_fast(x):
    q = x.shape[0] // 4
    s = (x[0:q] + x[q:2 * q]) + (x[2 * q:3 * q] + x[3 * q:])
    return jnp.sum(s, axis=0, keepdims=True) * (1.0 / x.shape[0])


def _colmean(x):
    return jnp.sum(x, axis=0, keepdims=True) * (1.0 / x.shape[0])


def _ln_t(x, fast=False):
    mean = _colmean_fast if fast else _colmean
    xc = x - mean(x)
    v = mean(xc * xc)
    return xc * lax.rsqrt(v + EPS)


def _kernel(x_hbm, wqkv_hbm, wo_hbm, w1_hbm, w2t_hbm, b1_hbm, b2_hbm,
            o_hbm,
            x_v, wqkv_v, wo_v, w1_v, w2t_v, wall_t, wot, b2c,
            k_scr, vt_scr, qm_scr, s_scr, otn_scr, o_v, xn_scr, done_scr,
            b1_v, b2_v, sems):
    i = pl.program_id(0)
    osem = sems.at[6]

    @pl.when(i == 0)
    def _prologue():
        def xcopy(lo, hi, sem):
            return pltpu.make_async_copy(x_hbm.at[:, lo:hi], x_v.at[:, lo:hi], sem)

        def wcopy(p, sem):
            lo, hi = WPIECES[p]
            return pltpu.make_async_copy(wqkv_hbm.at[:, lo:hi], wqkv_v.at[:, lo:hi], sem)

        th = TP // 2
        stage = [
            [xcopy(0, th, sems.at[0])],
            [wcopy(0, sems.at[1])],
            [wcopy(1, sems.at[2]), xcopy(th, TP, sems.at[2])],
            [wcopy(2, sems.at[3])],
            [xcopy(TP, S, sems.at[4]), pltpu.make_async_copy(wo_hbm, wo_v, sems.at[4]),
             pltpu.make_async_copy(b2_hbm, b2_v, sems.at[4])],
            [pltpu.make_async_copy(src, dst, sems.at[5])
             for src, dst in ((w1_hbm, w1_v), (b1_hbm, b1_v), (w2t_hbm, w2t_v))],
        ]
        for st in stage:
            for cp in st:
                cp.start()

        def wait(k):
            for cp in stage[k]:
                cp.wait()

        def prep_w(p):
            lo, hi = WPIECES[p]
            wt = wqkv_v[:, lo:hi].T
            wall_t[lo:hi, :] = wt
            return wt

        r4 = lax.broadcasted_iota(jnp.int32, (DP - DH, TP), 0)
        vpad = jnp.where(r4 == 0, 1.0, 0.0)
        kpad = jnp.zeros((128 - G, TP), bf16)

        def proj(c, lo, hi, xn=None, t0=0, t1=TP, w=None):
            if xn is None:
                xn = xn_scr[:, c * TP + t0:c * TP + t1]
            r = _dot(wall_t[lo:hi, :] if w is None else w, xn)
            roww = lax.broadcasted_iota(jnp.int32, (QW, t1 - t0), 0)
            for g in range(4):
                if lo <= G * g < hi:
                    for j in range(4):
                        o = G * g + QOFF[j] - lo
                        b = DH * j - QOFF[j]
                        msk = (roww >= b) & (roww < b + DH)
                        qw = jnp.where(msk, r[o:o + QW, :] * QSCALE, 0.0)
                        for l in range((t1 - t0) // 128):
                            qm_scr[(c * TP + t0) // 128 + l, 4 * g + j] = (
                                qw[:, l * 128:(l + 1) * 128].astype(bf16))
            for g in range(4):
                if lo <= D + G * g < hi:
                    o = D + G * g - lo
                    kg = jnp.concatenate([r[o:o + G, :].astype(bf16), kpad], axis=0)
                    k_scr[g, c * TP:(c + 1) * TP, :] = kg.T
            for h in range(H):
                if lo <= 2 * D + DH * h < hi:
                    o = 2 * D + DH * h - lo
                    vt = jnp.concatenate([r[o:o + DH, :], vpad], axis=0)
                    for l in range(TP // 128):
                        vt_scr[c * TP // 128 + l, h] = vt[:, l * 128:(l + 1) * 128].astype(bf16)

        def ln_tile(c0):
            return _ln_t(x_v[:, c0:c0 + 128].astype(f32), c0 < th).astype(bf16)

        def ln_store(lo, hi):
            for c0 in range(lo, hi, 128):
                xn_scr[:, c0:c0 + 128] = ln_tile(c0)

        s_scr[0:8, :] = jnp.zeros((8, 512), f32)
        done_scr[0:8, :] = jnp.zeros((8, 512), f32)
        otn_scr[0, 0:16, :] = jnp.zeros((16, 128), bf16)

        wait(0)
        ln_store(0, th)
        wait(1)
        wt = prep_w(0)
        proj(0, 0, G, None, 0, th, wt[0:G])
        wait(2)
        proj(0, G, 2 * G, None, 0, th)
        prep_w(1)
        proj(0, 2 * G, D, None, 0, th)
        ln_store(th, TP)
        proj(0, 0, 3 * G, None, th, TP)
        wait(3)
        proj(0, 3 * G, D, None, th, TP)
        prep_w(2)
        proj(0, D, 2 * D)
        proj(0, 2 * D, 3 * D - G)
        wait(4)
        proj(0, 3 * D - G, 3 * D)
        for c in range(1, NP):
            xn = jnp.concatenate([ln_tile(c0) for c0 in range(c * TP, (c + 1) * TP, 128)], axis=1)
            proj(c, 0, 3 * D, xn)

        wo32 = wo_v[...].astype(f32)
        zpad = jnp.zeros((DP - DH, D), f32)
        blks = []
        for h in range(H):
            blks.append(wo32[DH * h:DH * (h + 1), :])
            blks.append(zpad)
        wot[...] = jnp.concatenate(blks, axis=0).astype(bf16).T
        b2row = b2_v[...].reshape(1, D).astype(f32)
        b2c[...] = jnp.broadcast_to(b2row, (128, D)).T
        wait(5)

    q0s = [pl.multiple_of((i * NT + e) * 128, 128) for e in range(NT)]

    def qk_chunk(e, g, ga, m):
        c = ga % NC
        cols = []
        for j in range(4):
            parts = []
            if QOFF[j]:
                parts.append(jnp.zeros((QOFF[j], 128), bf16))
            parts.append(qm_scr[i * NT + e, 4 * g + j])
            parts.append(jnp.zeros((128 - QW - QOFF[j], 128), bf16))
            cols.append(jnp.concatenate(parts, axis=0))
        s = _dot(k_scr[g, c * CK:(c + 1) * CK, :], jnp.concatenate(cols, axis=1))
        sl = ga % NSLOT
        s_scr[sl * CK:(sl + 1) * CK, :] = s
        sm = jnp.max(s.reshape(CK // 8, 8, 512), axis=0)
        return sm if m is None else jnp.maximum(m, sm)

    def pv_chunk(g, gb, m_old, m, acc):
        c = gb % NC
        sl = gb % NSLOT
        if acc is not None:
            acc = acc * jnp.exp2(m_old - m)
        p = jnp.exp2(s_scr[sl * CK:(sl + 1) * CK, :] - m)
        o = jnp.concatenate(
            [_dot(vt_scr[c, 4 * g + j], p[:, j * 128:(j + 1) * 128].astype(bf16))
             for j in range(4)], axis=1)
        return o if acc is None else acc + o

    def finish(u, o):
        e, g = divmod(u, 4)
        on = (o * (1.0 / o[DH:DH + 1, :])).astype(bf16)
        for j in range(4):
            otn_scr[e, (4 * g + j) * DP:(4 * g + j + 1) * DP, :] = on[:, j * 128:(j + 1) * 128]

    hs = {}
    hns = {}
    rs = {}

    def st_wo(e):
        attn = _dot(wot[...], otn_scr[e])
        hs[e] = x_v[:, pl.ds(q0s[e], 128)].astype(f32) + attn
        hns[e] = _ln_t(hs[e]).astype(bf16).T

    def st_f1(e, lo=0, hi=F):
        b1row = b1_v[...].reshape(1, F).astype(f32)
        h1 = jnp.maximum(_dot(hns[e], w1_v[:, lo:hi]) + b1row[:, lo:hi], 0.0)
        rs.setdefault(e, []).append((h1 * h1).astype(bf16))

    def st_f2(e):
        out = lax.dot_general(w2t_v[...], jnp.concatenate(rs[e], axis=1),
                              (((1,), (1,)), ((), ())), preferred_element_type=f32)
        o_v[:, pl.ds(q0s[e], 128)] = (hs[e] + b2c[...] + out).astype(bf16)
        pltpu.make_async_copy(o_v.at[:, pl.ds(q0s[e], 128)], o_hbm.at[:, pl.ds(q0s[e], 128)],
                              osem).start()

    mrun = {}
    accs = {}
    NU = 4 * NT
    NG = NU * NC

    def do_pv(gb):
        u, c = divmod(gb, NC)
        accs[u] = pv_chunk(u % 4, gb, mrun.get(gb - 1), mrun[gb], accs.get(u))
        if c == FINISH_AT and u >= 1:
            finish(u - 1, done_scr[...])
        if c == NC - 1 and u < NU - 1:
            done_scr[...] = accs[u]
        if c == WO_AT and u % 4 == 0 and u >= 4:
            st_wo(u // 4 - 1)

    m8 = None
    for ga in range(NG):
        u, c = divmod(ga, NC)
        m8 = qk_chunk(u // 4, u % 4, ga, m8 if c else None)
        mrun[ga] = jnp.max(m8, axis=0, keepdims=True)
        if ga >= LAG:
            do_pv(ga - LAG)
    npc = LAG + 2
    bounds = [(F // 128 * k // npc) * 128 for k in range(npc + 1)]
    for k in range(npc):
        st_f1(0, bounds[k], bounds[k + 1])
        if k < LAG:
            do_pv(NG - LAG + k)
        if k == LAG - 1:
            finish(NU - 1, accs[NU - 1])
        if k == LAG:
            st_wo(NT - 1)
    for e in range(1, NT - 1):
        st_f1(e)
    for e in range(NT - 1):
        st_f2(e)
    st_f1(NT - 1)
    st_f2(NT - 1)

    @pl.when(i == NB - 1)
    def _drain():
        pltpu.make_async_copy(o_v, o_hbm, osem).wait()


@jax.jit
def pallas_sequential_preLN__mha_block__dense_activation_squared_relu__prompt_kernel(
    A_x: jax.Array,
    A_wqkv: jax.Array,
    A_wo: jax.Array,
    B_x: jax.Array,
    B_w1: jax.Array,
    B_b1: jax.Array,
    B_w2: jax.Array,
    B_b2: jax.Array,
):
    del B_x
    xt = A_x.reshape(S, D).T
    w2t = B_w2.T
    anyspec = pl.BlockSpec(memory_space=pl.ANY)
    out_t = pl.pallas_call(
        _kernel,
        grid=(NB,),
        in_specs=[anyspec] * 7,
        out_specs=anyspec,
        out_shape=jax.ShapeDtypeStruct((D, S), bf16),
        scratch_shapes=[
            pltpu.VMEM((D, S), bf16),
            pltpu.VMEM((D, 3 * D), bf16),
            pltpu.VMEM((D, D), bf16),
            pltpu.VMEM((D, F), bf16),
            pltpu.VMEM((D, F), bf16),
            pltpu.VMEM((3 * D, D), bf16),
            pltpu.VMEM((D, H * DP), bf16),
            pltpu.VMEM((D, 128), f32),
            pltpu.VMEM((4, S, 128), bf16),
            pltpu.VMEM((NC, H, DP, 128), bf16),
            pltpu.VMEM((S // 128, H, QW, 128), bf16),
            pltpu.VMEM((NSLOT * CK, 512), f32),
            pltpu.VMEM((NT, H * DP, 128), bf16),
            pltpu.VMEM((D, S), bf16),
            pltpu.VMEM((D, TP), bf16),
            pltpu.VMEM((DP, 512), f32),
            pltpu.VMEM((F,), bf16),
            pltpu.VMEM((D,), bf16),
            pltpu.SemaphoreType.DMA((7,)),
        ],
        compiler_params=pltpu.CompilerParams(
            dimension_semantics=("arbitrary",), vmem_limit_bytes=100 * 1024 * 1024,
            disable_bounds_checks=True, disable_semaphore_checks=True),
    )(xt, A_wqkv, A_wo, B_w1, w2t, B_b1, B_b2)
    return out_t.T.reshape(1, S, D)
```
